```python
import jax
import jax.numpy as jnp

def _softmax(x, axis=-1):
    return jax.nn.softmax(x, axis=axis)

def _gelu(x):
    return jax.nn.gelu(x, approximate=True)

def _silu(x):
    return jax.nn.silu(x)

def _sigmoid(x):
    return jax.nn.sigmoid(x)

def _layernorm(x, axis=-1, eps=1e-05):
    m = jnp.mean(x, axis=axis, keepdims=True)
    v = jnp.var(x, axis=axis, keepdims=True)
    return (x - m) / jnp.sqrt(v + eps)

def _scatter_add(tgt, idx, src, axis=0):
    return tgt.at[idx].add(src)

def _segment_sum(src, seg, n):
    return jax.ops.segment_sum(src, seg, n)

class _Rng:

    def __init__(self, key):
        self._k = key

    def _next(self):
        self._k, sub = jax.random.split(self._k)
        return sub

    def normal(self, shape):
        return jax.random.normal(self._next(), shape, dtype=jnp.bfloat16)

    def randint(self, lo, hi, shape):
        return jax.random.randint(self._next(), shape, lo, hi, dtype=jnp.int32)

    def uniform(self, shape, lo=0.0, hi=1.0):
        return jax.random.uniform(self._next(), shape, jnp.bfloat16, lo, hi)

    def permutation(self, n):
        return jax.random.permutation(self._next(), n)
kernel_name = 'recurrent_scan__ssm_conv_h3__mixer_gmlp__prompt'

def setup_inputs():
    _rng = _Rng(jax.random.key(int.from_bytes(__import__("os").urandom(4), "little")))
    _w = lambda a: (lambda t: t.astype(jnp.bfloat16) if jnp.issubdtype(t.dtype, jnp.floating) else t)(jnp.asarray(a))

    def _A_setup():
        B, S, D = (1, 2048, 640)
        ks = 4
        return {'q': _w((lambda *s: _rng.normal(s) * 0.05)(B, S, D)), 'k': _w((lambda *s: _rng.normal(s) * 0.05)(B, S, D)), 'v': _w((lambda *s: _rng.normal(s) * 0.05)(B, S, D)), 'shift_k': _w((lambda *s: _rng.normal(s) * 0.05)(D, ks) * 0.5), 'ssm_k': _w((lambda *s: _rng.normal(s) * 0.05)(D, S) * (1.0 / S ** 0.5)), 'ssm_D': _w((lambda *s: _rng.normal(s) * 0.05)(D))}
    _A_in = _A_setup()

    def _B_setup():
        B, S, D, F = (1, 2048, 640, 1536)
        Fh = F // 2
        return {'x': _w((lambda *s: _rng.normal(s) * 0.05)(B, S, D)), 'w_in': _w((lambda *s: _rng.normal(s) * 0.05)(D, 2 * Fh)), 'w_sp': _w(0.01 * (lambda *s: _rng.normal(s) * 0.05)(S, S)), 'b_sp': _w(1.0 + 0.01 * (lambda *s: _rng.normal(s) * 0.05)(S)), 'w_out': _w((lambda *s: _rng.normal(s) * 0.05)(Fh, D))}
    _B_in = _B_setup()
    return {'A_q': _A_in['q'], 'A_k': _A_in['k'], 'A_v': _A_in['v'], 'A_shift_k': _A_in['shift_k'], 'A_ssm_k': _A_in['ssm_k'], 'A_ssm_D': _A_in['ssm_D'], 'B_x': _B_in['x'], 'B_w_in': _B_in['w_in'], 'B_w_sp': _B_in['w_sp'], 'B_b_sp': _B_in['b_sp'], 'B_w_out': _B_in['w_out']}

def reference(A_q, A_k, A_v, A_shift_k, A_ssm_k, A_ssm_D, B_x, B_w_in, B_w_sp, B_b_sp, B_w_out):

    def _A_ref(q, k, v, shift_k, ssm_k, ssm_D):
        B, S, D = q.shape
        ks = shift_k.shape[-1]
        k_pad = jnp.pad(k, ((0, 0), (ks - 1, 0), (0, 0)))
        k_shift = jnp.zeros_like(k)
        for t in range(ks):
            k_shift = k_shift + k_pad[:, t:t + S, :] * shift_k[:, ks - 1 - t][None, None, :]
        kv = k_shift * v
        L = 2 * S
        kv_pad = jnp.pad(kv, ((0, 0), (0, S), (0, 0)))
        kf_pad = jnp.pad(ssm_k, ((0, 0), (0, S)))
        kv_f = (lambda x, axes=(-2, -1): jnp.fft.rfft2(x.astype(jnp.float32), axes=axes))(kv_pad[:, None, :, :], axes=(1, 2))
        kf_f = (lambda x, axes=(-2, -1): jnp.fft.rfft2(x.astype(jnp.float32), axes=axes))(kf_pad[:, None, :], axes=(1, 2))
        kf_f = (lambda x, *d: x.transpose(*d))(kf_f, 1, 2, 0)
        y_f = kv_f * kf_f[None, :, :, :]
        y = (lambda x, s, axes=(-2, -1): jnp.fft.irfft2(x, s=s, axes=axes).astype(jnp.bfloat16))(y_f, (1, L), axes=(1, 2))[:, 0, :S, :]
        y = y + kv * ssm_D[None, None, :]
        return q * y

    def _B_ref(x, w_in, w_sp, b_sp, w_out):
        B, S, D = x.shape
        F = w_in.shape[-1]
        Fh = F // 2
        z = _gelu(jnp.einsum('bsd,df->bsf', x, w_in))
        z1 = z[..., :Fh].copy()
        z2 = _layernorm(z[..., Fh:], axis=-1)
        g = jnp.einsum('ts,bsf->btf', w_sp, z2) + b_sp[None, :, None]
        return jnp.einsum('bsf,fd->bsd', z1 * g, w_out)
    x = A_q
    xn = _layernorm(x, axis=-1)
    s = _A_ref(xn, A_k, A_v, A_shift_k, A_ssm_k, A_ssm_D)
    g = _silu(_B_ref(xn, B_w_in, B_w_sp, B_b_sp, B_w_out))
    return x + s * g
```

```python
import math

import numpy as np
import ml_dtypes

import jax
import jax.numpy as jnp
from jax import lax
import jax.experimental.pallas as pl
import jax.experimental.pallas.tpu as pltpu

S_LEN = 2048
D_MODEL = 640
F_HALF = 768
NC = D_MODEL // 128
RT = 256
NRT = S_LEN // RT

_C8 = math.cos(math.pi / 8)
_S8 = math.sin(math.pi / 8)
_R2 = math.sqrt(0.5)


def _dft_tables():
    k2 = np.arange(64)[:, None].astype(np.float64)
    n2 = np.arange(64)[None, :].astype(np.float64)
    fw, bw = [], []
    for j in range(32):
        f = np.exp(-2j * np.pi * (n2 * k2 / 64 + n2 * (2 * j + 0.5) / 4096))
        m = np.block([[f.real, -f.imag], [f.imag, f.real]])
        fw.append(m)
        bw.append(m.T * (2.0 / 4096))
    fw = np.stack(fw).astype(np.float32).astype(ml_dtypes.bfloat16)
    bw = np.stack(bw).astype(np.float32).astype(ml_dtypes.bfloat16)
    return fw, bw


_FW_TAB, _BW_TAB = _dft_tables()


def _cmul_const(a, b, ang):
    wr, wi = math.cos(ang), math.sin(ang)
    return a * wr - b * wi, a * wi + b * wr


def _pass_a(x0, x1, x2, x3, b):
    cp = x2 * _R2
    cx1 = x1 * _C8
    sx1 = x1 * _S8
    cx3 = x3 * _C8
    sx3 = x3 * _S8
    p = cx1 + sx3
    q = sx1 + cx3
    r = cx3 - sx1
    t = sx3 - cx1
    e = x0 + cp
    o = x0 - cp
    outs = [(e + p, -(cp + q)), (o + r, cp + t), (e - p, q - cp), (o - r, cp - t)]
    if b == 0:
        return outs
    res = []
    for j, (a, bb) in enumerate(outs):
        if j == 0:
            m = cp + q
            ang = -math.pi * b * (1 + 4 * j) / 64
            wr, wi = math.cos(ang), math.sin(ang)
            res.append((a * wr + m * wi, a * wi - m * wr))
        else:
            res.append(_cmul_const(a, bb, -math.pi * b * (1 + 4 * j) / 64))
    return res


def _pass_a_inv(ins, b):
    z = ins if b == 0 else [
        _cmul_const(a, bb, math.pi * b * (1 + 4 * j) / 64) for j, (a, bb) in enumerate(ins)
    ]
    (a0, b0), (a1, b1), (a2, b2), (a3, b3) = z
    e = a0 + a2
    p = a0 - a2
    o = a1 + a3
    r = a1 - a3
    q = b2 - b0
    t = b1 - b3
    cp = (e - o) + ((b1 + b3) - (b0 + b2))
    x0 = e + o
    x2 = cp * _R2
    x1 = (p - t) * _C8 + (q - r) * _S8
    x3 = (p + t) * _S8 + (q + r) * _C8
    return x0, x1, x2, x3


def _radix8(a, inv):
    def add(x, y):
        return (x[0] + y[0], x[1] + y[1])

    def sub(x, y):
        return (x[0] - y[0], x[1] - y[1])

    def add_mi(x, y):
        return (x[0] + y[1], x[1] - y[0]) if not inv else (x[0] - y[1], x[1] + y[0])

    def sub_mi(x, y):
        return (x[0] - y[1], x[1] + y[0]) if not inv else (x[0] + y[1], x[1] - y[0])

    b0, b1 = add(a[0], a[4]), sub(a[0], a[4])
    b2, b3 = add(a[2], a[6]), sub(a[2], a[6])
    b4, b5 = add(a[1], a[5]), sub(a[1], a[5])
    b6, b7 = add(a[3], a[7]), sub(a[3], a[7])
    e02p, e02m = add(b0, b2), sub(b0, b2)
    e13p, e13m = add(b4, b6), sub(b4, b6)
    x0, x4 = add(e02p, e13p), sub(e02p, e13p)
    x2, x6 = add_mi(e02m, e13m), sub_mi(e02m, e13m)
    o02p, o02m = add_mi(b1, b3), sub_mi(b1, b3)
    cc, dd = add(b5, b7), sub(b5, b7)
    if not inv:
        o13p = ((dd[0] + cc[1]) * _R2, (dd[1] - cc[0]) * _R2)
        o13m = ((cc[0] + dd[1]) * _R2, (cc[1] - dd[0]) * _R2)
    else:
        o13p = ((dd[0] - cc[1]) * _R2, (dd[1] + cc[0]) * _R2)
        o13m = ((cc[0] - dd[1]) * _R2, (cc[1] + dd[0]) * _R2)
    x1, x5 = add(o02p, o13p), sub(o02p, o13p)
    x3, x7 = add_mi(o02m, o13m), sub_mi(o02m, o13m)
    return [x0, x1, x2, x3, x4, x5, x6, x7]


def _ln(x, eps=1e-5):
    m = jnp.mean(x, axis=-1, keepdims=True)
    xc = x - m
    v = jnp.mean(xc * xc, axis=-1, keepdims=True)
    return xc * lax.rsqrt(v + eps)


def _gelu(x):
    c = math.sqrt(2.0 / math.pi)
    return 0.5 * x * (1.0 + jnp.tanh(c * (x + 0.044715 * (x * x * x))))


def _kernel(x_hbm, k_hbm, v_hbm, shk_hbm, ssmk_hbm, ssmd_hbm, win_hbm, wsp_hbm, bsp_hbm,
            wout_hbm, fw_hbm, bw_hbm,
            out_hbm,
            x_v, k_v, v_v, shk_v, ssmk_v, ssmd_v, win_v, wsp_v, bsp_v, wout_v, fw_v, bw_v,
            xn_v, z1_v, z2_v, kpad_v, kv_v, kt_v, t_v, au_v, ak_v, b_v, y_v, gate_v, ob_v,
            sem_x, sem_kv, sem_w, sem_sp, sem_o):
    f32, bf16 = jnp.float32, jnp.bfloat16

    def x_cp(i):
        return pltpu.make_async_copy(x_hbm.at[pl.ds(i * RT, RT)], x_v.at[pl.ds(i * RT, RT)], sem_x.at[i])

    def k_cp(i):
        return pltpu.make_async_copy(k_hbm.at[pl.ds(i * RT, RT)], k_v.at[pl.ds(i * RT, RT)], sem_kv.at[0, i])

    def v_cp(i):
        return pltpu.make_async_copy(v_hbm.at[pl.ds(i * RT, RT)], v_v.at[pl.ds(i * RT, RT)], sem_kv.at[1, i])

    def sp_cp(i):
        return pltpu.make_async_copy(wsp_hbm.at[pl.ds(i * RT, RT)], wsp_v.at[pl.ds(i * RT, RT)], sem_sp.at[i])

    w_cps = [
        pltpu.make_async_copy(win_hbm, win_v, sem_w.at[0]),
        pltpu.make_async_copy(shk_hbm, shk_v, sem_w.at[1]),
        pltpu.make_async_copy(ssmd_hbm, ssmd_v, sem_w.at[2]),
        pltpu.make_async_copy(bsp_hbm, bsp_v, sem_w.at[3]),
        pltpu.make_async_copy(ssmk_hbm, ssmk_v, sem_w.at[4]),
        pltpu.make_async_copy(fw_hbm, fw_v, sem_w.at[5]),
        pltpu.make_async_copy(bw_hbm, bw_v, sem_w.at[6]),
        pltpu.make_async_copy(wout_hbm, wout_v, sem_w.at[7]),
    ]

    x_cp(0).start()
    w_cps[0].start()
    k_cp(0).start()
    v_cp(0).start()
    w_cps[1].start()
    w_cps[2].start()
    w_cps[3].start()

    kpad_v[pl.ds(0, 8), :] = jnp.zeros((8, D_MODEL), f32)

    w_cps[0].wait()
    w_cps[1].wait()
    w_cps[2].wait()
    w_cps[3].wait()

    def p1_body(i, carry):
        @pl.when(i + 1 < NRT)
        def _():
            x_cp(i + 1).start()
            k_cp(i + 1).start()
            v_cp(i + 1).start()

        for step, which in ((0, 4), (1, 5), (2, 6), (3, 7)):
            @pl.when(i == step)
            def _():
                w_cps[which].start()

        @pl.when(i >= 4)
        def _():
            sp_cp(2 * (i - 4)).start()
            sp_cp(2 * (i - 4) + 1).start()

        x_cp(i).wait()
        r0 = pl.multiple_of(i * RT, RT)
        rows = pl.ds(r0, RT)
        xn = _ln(x_v[rows, :].astype(f32)).astype(bf16)
        xn_v[rows, :] = xn
        z = jnp.dot(xn, win_v[...], preferred_element_type=f32)
        z = _gelu(z)
        z1_v[rows, :] = z[:, :F_HALF].astype(bf16)
        z2_v[rows, :] = _ln(z[:, F_HALF:]).astype(bf16)

        k_cp(i).wait()
        v_cp(i).wait()
        kpad_v[pl.ds(r0 + 8, RT), :] = k_v[rows, :].astype(f32)
        big = kpad_v[pl.ds(r0, RT + 8), :]
        ks = big[8:] * shk_v[0:1, :]
        for j in range(1, 4):
            ks = ks + big[8 - j:8 - j + RT] * shk_v[j:j + 1, :]
        kv = ks * v_v[rows, :].astype(f32)
        for c in range(NC):
            kv_v[c, rows, :] = kv[:, c * 128:(c + 1) * 128]
        return carry

    lax.fori_loop(0, NRT, p1_body, 0)

    w_cps[4].wait()

    def kt_body(i, carry):
        r0 = pl.multiple_of(i * RT, RT)
        for c in range(NC):
            blk = ssmk_v[c * 128:(c + 1) * 128, pl.ds(r0, RT)].astype(f32)
            kt_v[c, pl.ds(r0, RT), :] = blk.T
        return carry

    lax.fori_loop(0, NRT, kt_body, 0)

    def s1(src, dst, c, g):
        r0 = pl.multiple_of(g * 16, 16)
        for b in range(8):
            xs = [src[c, pl.ds(64 * (b + 8 * h) + r0, 16), :] for h in range(4)]
            outs = _pass_a(*xs, b)
            for j in range(4):
                t_v[j, b, 0] = outs[j][0]
                t_v[j, b, 1] = outs[j][1]
        for j in range(4):
            o = _radix8([(t_v[j, b, 0], t_v[j, b, 1]) for b in range(8)], False)
            for m in range(8):
                dst[j + 4 * m, c, pl.ds(r0, 16), :] = o[m][0].astype(bf16)
                dst[j + 4 * m, c, pl.ds(64 + r0, 16), :] = o[m][1].astype(bf16)

    def s1_body(i, carry):
        c = i // 4
        g = i % 4
        s1(kv_v, au_v, c, g)
        s1(kt_v, ak_v, c, g)
        return carry

    lax.fori_loop(0, NC * 4, s1_body, 0)

    w_cps[5].wait()
    w_cps[6].wait()

    def s2_body(j, carry):
        fj = fw_v[j]
        gj = bw_v[j]
        for c in range(NC):
            u = jnp.dot(fj, au_v[j, c], preferred_element_type=f32)
            h = jnp.dot(fj, ak_v[j, c], preferred_element_type=f32)
            yr = u[:64] * h[:64] - u[64:] * h[64:]
            yi = u[:64] * h[64:] + u[64:] * h[:64]
            yy = jnp.concatenate([yr, yi], axis=0).astype(bf16)
            b_v[j, c] = jnp.dot(gj, yy, preferred_element_type=f32)
        return carry

    lax.fori_loop(0, 32, s2_body, 0)

    def s3_body(i, carry):
        c = i // 4
        g = i % 4
        r0 = pl.multiple_of(g * 16, 16)
        for j in range(4):
            ins = [(b_v[j + 4 * m, c, pl.ds(r0, 16), :], b_v[j + 4 * m, c, pl.ds(64 + r0, 16), :])
                   for m in range(8)]
            o = _radix8(ins, True)
            for b in range(8):
                t_v[j, b, 0] = o[b][0]
                t_v[j, b, 1] = o[b][1]
        for b in range(8):
            outs = _pass_a_inv([(t_v[j, b, 0], t_v[j, b, 1]) for j in range(4)], b)
            for h in range(4):
                y_v[c, pl.ds(64 * (b + 8 * h) + r0, 16), :] = outs[h]
        return carry

    lax.fori_loop(0, NC * 4, s3_body, 0)

    w_cps[7].wait()

    def o_cp(i, slot):
        return pltpu.make_async_copy(ob_v.at[slot], out_hbm.at[pl.ds(i * RT, RT)], sem_o.at[slot])

    def p2_body(i, carry):
        sp_cp(i).wait()
        r0 = pl.multiple_of(i * RT, RT)
        rows = pl.ds(r0, RT)
        g = jnp.dot(wsp_v[rows, :], z2_v[...], preferred_element_type=f32) + bsp_v[rows, :]
        t = (z1_v[rows, :].astype(f32) * g).astype(bf16)
        o = jnp.dot(t, wout_v[...], preferred_element_type=f32)
        gate = o * jax.nn.sigmoid(o)
        yc = jnp.concatenate([y_v[c, rows, :] + kv_v[c, rows, :] * ssmd_v[:, c * 128:(c + 1) * 128]
                              for c in range(NC)], axis=1)
        res = x_v[rows, :].astype(f32) + xn_v[rows, :].astype(f32) * yc * gate
        slot = i % 2

        @pl.when(i >= 2)
        def _():
            o_cp(i - 2, slot).wait()

        ob_v[slot] = res.astype(bf16)
        o_cp(i, slot).start()
        return carry

    lax.fori_loop(0, NRT, p2_body, 0)
    o_cp(NRT - 2, 0).wait()
    o_cp(NRT - 1, 1).wait()


@jax.jit
def pallas_recurrent_scan__ssm_conv_h3__mixer_gmlp__prompt_kernel(
    A_q: jax.Array,
    A_k: jax.Array,
    A_v: jax.Array,
    A_shift_k: jax.Array,
    A_ssm_k: jax.Array,
    A_ssm_D: jax.Array,
    B_x: jax.Array,
    B_w_in: jax.Array,
    B_w_sp: jax.Array,
    B_b_sp: jax.Array,
    B_w_out: jax.Array,
):
    del B_x
    b, s, d = A_q.shape
    assert (b, s, d) == (1, S_LEN, D_MODEL)
    f32, bf16 = jnp.float32, jnp.bfloat16
    x = A_q.reshape(s, d)
    k = A_k.reshape(s, d)
    v = A_v.reshape(s, d)
    shk = A_shift_k.T.astype(f32)
    ssmd = A_ssm_D.reshape(1, d).astype(f32)
    bsp = B_b_sp.reshape(s, 1).astype(f32)
    fw = jnp.asarray(_FW_TAB)
    bw = jnp.asarray(_BW_TAB)

    any_spec = pl.BlockSpec(memory_space=pl.ANY)
    vm = pltpu.VMEM
    scratch = [
        vm((s, d), bf16), vm((s, d), bf16), vm((s, d), bf16),
        vm((4, d), f32),
        vm((d, s), bf16),
        vm((1, d), f32),
        vm((d, 2 * F_HALF), bf16),
        vm((s, s), bf16),
        vm((s, 1), f32),
        vm((F_HALF, d), bf16),
        vm((32, 128, 128), bf16), vm((32, 128, 128), bf16),
        vm((s, d), bf16),
        vm((s, F_HALF), bf16), vm((s, F_HALF), bf16),
        vm((s + 8, d), f32),
        vm((NC, s, 128), f32),
        vm((NC, s, 128), f32),
        vm((4, 8, 2, 16, 128), f32),
        vm((32, NC, 128, 128), bf16), vm((32, NC, 128, 128), bf16),
        vm((32, NC, 128, 128), f32),
        vm((NC, s, 128), f32),
        vm((8, 128), f32),
        vm((2, RT, d), bf16),
        pltpu.SemaphoreType.DMA((NRT,)),
        pltpu.SemaphoreType.DMA((2, NRT)),
        pltpu.SemaphoreType.DMA((8,)),
        pltpu.SemaphoreType.DMA((NRT,)),
        pltpu.SemaphoreType.DMA((2,)),
    ]
    out = pl.pallas_call(
        _kernel,
        out_shape=jax.ShapeDtypeStruct((s, d), bf16),
        in_specs=[any_spec] * 12,
        out_specs=any_spec,
        scratch_shapes=scratch,
        compiler_params=pltpu.CompilerParams(vmem_limit_bytes=110 * 1024 * 1024),
    )(x, k, v, shk, A_ssm_k, ssmd, B_w_in, B_w_sp, bsp, B_w_out, fw, bw)
    return out.reshape(b, s, d)
```

```python
import math
import functools

import numpy as np
import ml_dtypes

import jax
import jax.numpy as jnp
from jax import lax
import jax.experimental.pallas as pl
import jax.experimental.pallas.tpu as pltpu

S_LEN = 2048
D_MODEL = 640
F_HALF = 768
NC = D_MODEL // 128
RT = 256
NRT = S_LEN // RT
KP = 128
KV0 = 0
KT0 = NC * S_LEN
T0 = 2 * NC * S_LEN
AU0 = T0 + 2 * 64 * 16
AK0 = AU0 + 32 * NC * 64
B0 = AK0 + 32 * NC * 64
Y0 = B0 + 32 * NC * 128
BIG_ROWS = Y0 + NC * S_LEN
KO = 128

_C8 = math.cos(math.pi / 8)
_S8 = math.sin(math.pi / 8)
_R2 = math.sqrt(0.5)


def _dft_tables():
    k2 = np.arange(64)[:, None].astype(np.float64)
    n2 = np.arange(64)[None, :].astype(np.float64)
    fw, bw = [], []
    for j in range(32):
        f = np.exp(-2j * np.pi * (n2 * k2 / 64 + n2 * (2 * j + 0.5) / 4096))
        m = np.block([[f.real, -f.imag], [f.imag, f.real]])
        perm = np.stack([np.arange(64), 64 + np.arange(64)], axis=1).reshape(-1)
        fw.append(m[:, perm])
        bw.append((m.T * (2.0 / 4096))[:, perm])
    fw = np.stack(fw).astype(np.float32).astype(ml_dtypes.bfloat16)
    bw = np.stack(bw).astype(np.float32).astype(ml_dtypes.bfloat16)
    return fw, bw


_FW_TAB, _BW_TAB = _dft_tables()


def _cmul_const(a, b, ang):
    wr, wi = math.cos(ang), math.sin(ang)
    return a * wr - b * wi, a * wi + b * wr


def _pass_a(x0, x1, x2, x3, b):
    cp = x2 * _R2
    cx1 = x1 * _C8
    sx1 = x1 * _S8
    cx3 = x3 * _C8
    sx3 = x3 * _S8
    p = cx1 + sx3
    q = sx1 + cx3
    r = cx3 - sx1
    t = sx3 - cx1
    e = x0 + cp
    o = x0 - cp
    outs = [(e + p, -(cp + q)), (o + r, cp + t), (e - p, q - cp), (o - r, cp - t)]
    if b == 0:
        return outs
    res = []
    for j, (a, bb) in enumerate(outs):
        if j == 0:
            m = cp + q
            ang = -math.pi * b * (1 + 4 * j) / 64
            wr, wi = math.cos(ang), math.sin(ang)
            res.append((a * wr + m * wi, a * wi - m * wr))
        else:
            res.append(_cmul_const(a, bb, -math.pi * b * (1 + 4 * j) / 64))
    return res


def _pass_a_inv(ins, b):
    z = ins if b == 0 else [
        _cmul_const(a, bb, math.pi * b * (1 + 4 * j) / 64) for j, (a, bb) in enumerate(ins)
    ]
    (a0, b0), (a1, b1), (a2, b2), (a3, b3) = z
    e = a0 + a2
    p = a0 - a2
    o = a1 + a3
    r = a1 - a3
    q = b2 - b0
    t = b1 - b3
    cp = (e - o) + ((b1 + b3) - (b0 + b2))
    x0 = e + o
    x2 = cp * _R2
    x1 = (p - t) * _C8 + (q - r) * _S8
    x3 = (p + t) * _S8 + (q + r) * _C8
    return x0, x1, x2, x3


def _radix8(a, inv):
    def add(x, y):
        return (x[0] + y[0], x[1] + y[1])

    def sub(x, y):
        return (x[0] - y[0], x[1] - y[1])

    def add_mi(x, y):
        return (x[0] + y[1], x[1] - y[0]) if not inv else (x[0] - y[1], x[1] + y[0])

    def sub_mi(x, y):
        return (x[0] - y[1], x[1] + y[0]) if not inv else (x[0] + y[1], x[1] - y[0])

    b0, b1 = add(a[0], a[4]), sub(a[0], a[4])
    b2, b3 = add(a[2], a[6]), sub(a[2], a[6])
    b4, b5 = add(a[1], a[5]), sub(a[1], a[5])
    b6, b7 = add(a[3], a[7]), sub(a[3], a[7])
    e02p, e02m = add(b0, b2), sub(b0, b2)
    e13p, e13m = add(b4, b6), sub(b4, b6)
    x0, x4 = add(e02p, e13p), sub(e02p, e13p)
    x2, x6 = add_mi(e02m, e13m), sub_mi(e02m, e13m)
    o02p, o02m = add_mi(b1, b3), sub_mi(b1, b3)
    cc, dd = add(b5, b7), sub(b5, b7)
    if not inv:
        o13p = ((dd[0] + cc[1]) * _R2, (dd[1] - cc[0]) * _R2)
        o13m = ((cc[0] + dd[1]) * _R2, (cc[1] - dd[0]) * _R2)
    else:
        o13p = ((dd[0] - cc[1]) * _R2, (dd[1] + cc[0]) * _R2)
        o13m = ((cc[0] - dd[1]) * _R2, (cc[1] + dd[0]) * _R2)
    x1, x5 = add(o02p, o13p), sub(o02p, o13p)
    x3, x7 = add_mi(o02m, o13m), sub_mi(o02m, o13m)
    return [x0, x1, x2, x3, x4, x5, x6, x7]


def _ln(x, eps=1e-5):
    m = jnp.mean(x, axis=-1, keepdims=True)
    xc = x - m
    v = jnp.mean(xc * xc, axis=-1, keepdims=True)
    return xc * lax.rsqrt(v + eps)


def _gelu(x):
    c = math.sqrt(2.0 / math.pi)
    h = 0.5 * x
    t = jnp.tanh(x * (c + (c * 0.044715) * (x * x)))
    return h + h * t


def _kernel(x_hbm, k_hbm, v_hbm, shk_hbm, ssmk_hbm, ssmd_hbm, win_hbm, wsp_hbm, bsp_hbm,
            wout_hbm, fw_hbm, bw_hbm,
            out_hbm,
            x_v, k_v, v_v, shk_v, ssmk_v, ssmd_v, win_v, wsp_v, bsp_v, wout_v, fw_v, bw_v,
            xn_v, z1_v, z2_v, ya_v, big_v, zi_s, za_v, zb_v, ob_v, gate_v,
            sem_x, sem_kv, sem_w, sem_sp, sem_o):
    f32, bf16 = jnp.float32, jnp.bfloat16

    def x_cp(i):
        return pltpu.make_async_copy(x_hbm.at[pl.ds(i * RT, RT)], x_v.at[pl.ds(i * RT, RT)], sem_x.at[i])

    def k_cp(i):
        return pltpu.make_async_copy(k_hbm.at[pl.ds(i * RT, RT)], k_v.at[pl.ds(i * RT, RT)], sem_kv.at[0, i])

    def v_cp(i):
        return pltpu.make_async_copy(v_hbm.at[pl.ds(i * RT, RT)], v_v.at[pl.ds(i * RT, RT)], sem_kv.at[1, i])

    def sp_cp(i):
        return pltpu.make_async_copy(wsp_hbm.at[pl.ds(i * RT, RT)], wsp_v.at[pl.ds(i * RT, RT)], sem_sp.at[i])

    w_cps = [
        pltpu.make_async_copy(win_hbm, win_v, sem_w.at[0]),
        pltpu.make_async_copy(shk_hbm, shk_v, sem_w.at[1]),
        pltpu.make_async_copy(ssmd_hbm, ssmd_v, sem_w.at[2]),
        pltpu.make_async_copy(bsp_hbm, bsp_v, sem_w.at[3]),
        pltpu.make_async_copy(ssmk_hbm, ssmk_v, sem_w.at[4]),
        pltpu.make_async_copy(fw_hbm, fw_v, sem_w.at[5]),
        pltpu.make_async_copy(bw_hbm, bw_v, sem_w.at[6]),
        pltpu.make_async_copy(wout_hbm, wout_v, sem_w.at[7]),
    ]

    x_cp(0).start()
    w_cps[0].start()
    k_cp(0).start()
    v_cp(0).start()
    w_cps[1].start()
    w_cps[2].start()
    w_cps[3].start()


    w_cps[1].wait()
    w_cps[2].wait()
    w_cps[3].wait()

    CH = 32
    CC = 16

    zi_s[0] = 0

    def opq(v):
        return pl.multiple_of(zi_s[0] + v, 8)

    KP0 = RT + 8

    def st_a(i, zz):
        if i == 0:
            halo = jnp.zeros((8, D_MODEL), f32)
        else:
            halo = k_v[pl.ds(i * RT - 16, 16), :].astype(f32)[8:]
        zz[pl.ds(opq(KP0), 8), :D_MODEL] = halo
        for q in range(RT // CH):
            r0 = i * RT + q * CH
            rows = pl.ds(r0, CH)
            xn_v[rows, :] = _ln(x_v[rows, :].astype(f32)).astype(bf16)
            zz[pl.ds(opq(KP0 + 8 + q * CH), CH), :D_MODEL] = k_v[rows, :].astype(f32)
            big = zz[pl.ds(opq(KP0 + q * CH), CH + 8), :D_MODEL]
            ks = big[8:] * shk_v[0:1, :]
            for j in range(1, 4):
                ks = ks + big[8 - j:8 - j + CH] * shk_v[j:j + 1, :]
            kv = ks * v_v[rows, :].astype(f32)
            for c in range(NC):
                big_v[pl.ds(KV0 + c * S_LEN + r0, CH), :] = kv[:, c * 128:(c + 1) * 128]
            zz[pl.ds(opq(RT), 8), :128] = kv[:8, :128]

    def st_b(i, zz):
        rows = pl.ds(i * RT, RT)
        zz[:RT, :] = jnp.dot(xn_v[rows, :], win_v[...], preferred_element_type=f32)

    def st_c(i, zz):
        for q in range(RT // CC):
            rows = pl.ds(i * RT + q * CC, CC)
            rr = pl.ds(opq(q * CC), CC)
            z1_v[rows, :] = _gelu(zz[rr, :F_HALF]).astype(bf16)
            z2 = _ln(_gelu(zz[rr, F_HALF:]))
            z2_v[rows, :] = z2.astype(bf16)
            zz[pl.ds(opq(RT), 8), :128] = z2[:8, :128]

    def in_wait(i):
        x_cp(i).wait()
        k_cp(i).wait()
        v_cp(i).wait()

    def in_start(i):
        x_cp(i).start()
        k_cp(i).start()
        v_cp(i).start()

    if True:
        in_start(1)
        in_wait(0)
        st_a(0, zb_v)
        in_start(2)
        w_cps[0].wait()
        for i in range(NRT + 1):
            if i + 3 < NRT:
                in_start(i + 3)
            if i in (1, 3, 5, 7):
                w_cps[{1: 4, 3: 5, 5: 7, 7: 6}[i]].start()
            if i == 6:
                sp_cp(0).start()
            if i == NRT:
                sp_cp(1).start()
            if i + 1 < NRT:
                in_wait(i + 1)
            zw, zr = (za_v, zb_v) if i % 2 == 0 else (zb_v, za_v)
            if i >= 1:
                st_c(i - 1, zr)
            if i + 1 < NRT:
                st_a(i + 1, zr)
            if i < NRT:
                st_b(i, zw)

    w_cps[4].wait()

    def kt_body(i, carry):
        r0 = pl.multiple_of(i * RT, RT)
        for c in range(NC):
            blk = ssmk_v[c * 128:(c + 1) * 128, pl.ds(r0, RT)].astype(f32)
            big_v[pl.ds(KT0 + c * S_LEN + r0, RT), :] = blk.T
        return carry

    if True:
        lax.fori_loop(0, NRT, kt_body, 0)

    def pk(a, b):
        return lax.bitcast_convert_type(pltpu.pack_elementwise([a, b], packed_dtype=bf16), f32)

    def s1_items(src, dst, c, g, ti):
        r0 = pl.multiple_of(g * 16, 16)

        def pa(b):
            xs = [big_v[pl.ds(src + c * S_LEN + 64 * (b + 8 * h) + r0, 16), :] for h in range(4)]
            outs = _pass_a(*xs, b)
            for j in range(4):
                big_v[pl.ds(T0 + ((ti) * 64 + j * 16 + b * 2 + 0) * 16, 16), :] = outs[j][0]
                big_v[pl.ds(T0 + ((ti) * 64 + j * 16 + b * 2 + 1) * 16, 16), :] = outs[j][1]

        def pb(j):
            o = _radix8([(big_v[pl.ds(T0 + ((ti) * 64 + j * 16 + b * 2 + 0) * 16, 16), :], big_v[pl.ds(T0 + ((ti) * 64 + j * 16 + b * 2 + 1) * 16, 16), :]) for b in range(8)], False)
            for m in range(8):
                base = dst + ((j + 4 * m) * NC + c) * 64
                big_v[pl.ds(pl.multiple_of(base + r0, 16), 16), :] = pk(o[m][0], o[m][1])

        return [functools.partial(pa, b) for b in range(8)] + [functools.partial(pb, j) for j in range(4)]

    def p2_tile(i):
        rows = pl.ds(pl.multiple_of(i * RT, RT), RT)
        g = jnp.dot(wsp_v[rows, :], z2_v[...], preferred_element_type=f32) + bsp_v[rows, :]
        t = (z1_v[rows, :].astype(f32) * g).astype(bf16)
        o = jnp.dot(t, wout_v[...], preferred_element_type=f32)
        hh = 0.5 * o
        gate_v[rows, :] = hh + hh * jnp.tanh(hh)

    def interleave(a, b):
        na, nb = len(a), len(b)
        ia = ib = 0
        while ia < na or ib < nb:
            if ib >= nb or (ia < na and (ia + 0.5) * nb <= (ib + 0.5) * na):
                a[ia]()
                ia += 1
            else:
                b[ib]()
                ib += 1

    def s1_body(g, carry):
        sp_cp(g + 2).start()
        sp_cp(g).wait()
        items = []
        for c in range(NC):
            items += s1_items(KV0, AU0, c, g, 0)
            items += s1_items(KT0, AK0, c, g, 1)
        for it in items:
            it()
        p2_tile(g)
        return carry

    w_cps[7].wait()
    if True:
        lax.fori_loop(0, 4, s1_body, 0)

    w_cps[5].wait()
    w_cps[6].wait()

    def ld_a(base, j, c):
        return pltpu.bitcast(big_v[pl.ds(pl.multiple_of(base + (j * NC + c) * 64, 64), 64), :], bf16)

    def s2_body(j, carry):
        fj = fw_v[j]
        for c in range(NC):
            uh = jnp.dot(fj, jnp.concatenate([ld_a(AU0, j, c), ld_a(AK0, j, c)], axis=1), preferred_element_type=f32)
            u = uh[:, :128]
            h = uh[:, 128:]
            yr = u[:64] * h[:64] - u[64:] * h[64:]
            yi = u[:64] * h[64:] + u[64:] * h[:64]
            ya_v[pl.ds(pl.multiple_of((j * NC + c) * 64, 64), 64), :] = pk(yr, yi)
        return carry

    if True:
        lax.fori_loop(0, 32, s2_body, 0)

    def s2b_body(jj, carry):
        for j in (2 * jj, 2 * jj + 1):
            gj = bw_v[j]
            bb = jnp.dot(gj, jnp.concatenate([pltpu.bitcast(ya_v[pl.ds(pl.multiple_of((j * NC + c) * 64, 64), 64), :], bf16) for c in range(NC)], axis=1), preferred_element_type=f32)
            for c in range(NC):
                big_v[pl.ds(pl.multiple_of(B0 + (j * NC + c) * 128, 128), 128), :] = bb[:, c * 128:(c + 1) * 128]
        return carry

    if True:
        lax.fori_loop(0, 16, s2b_body, 0)

    def s3_body(g, carry):
        @pl.when(g < 2)
        def _():
            sp_cp(g + 6).start()

        sp_cp(g + 4).wait()
        r0 = pl.multiple_of(g * 16, 16)

        def ib(c, j):
            ins = [(big_v[pl.ds(B0 + ((j + 4 * m) * NC + c) * 128 + r0, 16), :], big_v[pl.ds(B0 + ((j + 4 * m) * NC + c) * 128 + 64 + r0, 16), :])
                   for m in range(8)]
            o = _radix8(ins, True)
            for b in range(8):
                big_v[pl.ds(T0 + ((c % 2) * 64 + j * 16 + b * 2 + 0) * 16, 16), :] = o[b][0]
                big_v[pl.ds(T0 + ((c % 2) * 64 + j * 16 + b * 2 + 1) * 16, 16), :] = o[b][1]

        def ia(c, b):
            outs = _pass_a_inv([(big_v[pl.ds(T0 + ((c % 2) * 64 + j * 16 + b * 2 + 0) * 16, 16), :], big_v[pl.ds(T0 + ((c % 2) * 64 + j * 16 + b * 2 + 1) * 16, 16), :]) for j in range(4)], b)
            for h in range(4):
                big_v[pl.ds(Y0 + c * S_LEN + 64 * (b + 8 * h) + r0, 16), :] = outs[h]

        items = []
        for c in range(NC):
            items += [functools.partial(ib, c, j) for j in range(4)]
            items += [functools.partial(ia, c, b) for b in range(8)]
        for it in items:
            it()
        p2_tile(g + 4)
        return carry

    if True:
        lax.fori_loop(0, 4, s3_body, 0)

    def o_cp(i, slot):
        return pltpu.make_async_copy(ob_v.at[slot], out_hbm.at[pl.ds(i * RT, RT)], sem_o.at[slot])

    def p2_body(i, carry):
        slot = i % 2

        @pl.when(i >= 2)
        def _():
            o_cp(i - 2, slot).wait()

        for q in range(RT // CH):
            rows = pl.ds(pl.multiple_of(i * RT + q * CH, CH), CH)
            yc = jnp.concatenate([big_v[pl.ds(pl.multiple_of(Y0 + c * S_LEN + i * RT + q * CH, CH), CH), :] + big_v[pl.ds(pl.multiple_of(KV0 + c * S_LEN + i * RT + q * CH, CH), CH), :] * ssmd_v[:, c * 128:(c + 1) * 128]
                                  for c in range(NC)], axis=1)
            res = x_v[rows, :].astype(f32) + xn_v[rows, :].astype(f32) * yc * gate_v[rows, :]
            ob_v[slot, pl.ds(q * CH, CH), :] = res.astype(bf16)
        o_cp(i, slot).start()
        return carry

    if True:
        lax.fori_loop(0, NRT, p2_body, 0)
    o_cp(NRT - 2, 0).wait()
    o_cp(NRT - 1, 1).wait()


@jax.jit
def pallas_recurrent_scan__ssm_conv_h3__mixer_gmlp__prompt_kernel(
    A_q: jax.Array,
    A_k: jax.Array,
    A_v: jax.Array,
    A_shift_k: jax.Array,
    A_ssm_k: jax.Array,
    A_ssm_D: jax.Array,
    B_x: jax.Array,
    B_w_in: jax.Array,
    B_w_sp: jax.Array,
    B_b_sp: jax.Array,
    B_w_out: jax.Array,
):
    del B_x
    b, s, d = A_q.shape
    assert (b, s, d) == (1, S_LEN, D_MODEL)
    f32, bf16 = jnp.float32, jnp.bfloat16
    x = A_q.reshape(s, d)
    k = A_k.reshape(s, d)
    v = A_v.reshape(s, d)
    shk = A_shift_k.T.astype(f32)
    ssmd = A_ssm_D.reshape(1, d).astype(f32)
    bsp = B_b_sp.reshape(s, 1).astype(f32)
    fw = jnp.asarray(_FW_TAB)
    bw = jnp.asarray(_BW_TAB)

    any_spec = pl.BlockSpec(memory_space=pl.ANY)
    vm = pltpu.VMEM
    scratch = [
        vm((s, d), bf16), vm((s, d), bf16), vm((s, d), bf16),
        vm((4, d), f32),
        vm((d, s), bf16),
        vm((1, d), f32),
        vm((d, 2 * F_HALF), bf16),
        vm((s, s), bf16),
        vm((s, 1), f32),
        vm((F_HALF, d), bf16),
        vm((32, 128, 128), bf16), vm((32, 128, 128), bf16),
        vm((s, d), bf16),
        vm((s, F_HALF), bf16), vm((s, F_HALF), bf16),
        vm((32 * NC * 64, 128), f32),
        vm((BIG_ROWS, 128), f32),
        pltpu.SMEM((1,), jnp.int32),
        vm((2 * RT + 16, 2 * F_HALF), f32), vm((2 * RT + 16, 2 * F_HALF), f32),
        vm((2, RT, d), bf16),
        vm((s, d), f32),
        pltpu.SemaphoreType.DMA((NRT,)),
        pltpu.SemaphoreType.DMA((2, NRT)),
        pltpu.SemaphoreType.DMA((8,)),
        pltpu.SemaphoreType.DMA((NRT,)),
        pltpu.SemaphoreType.DMA((2,)),
    ]
    out = pl.pallas_call(
        _kernel,
        out_shape=jax.ShapeDtypeStruct((s, d), bf16),
        in_specs=[any_spec] * 12,
        out_specs=any_spec,
        scratch_shapes=scratch,
        compiler_params=pltpu.CompilerParams(vmem_limit_bytes=110 * 1024 * 1024),
    )(x, k, v, shk, A_ssm_k, ssmd, B_w_in, B_w_sp, bsp, B_w_out, fw, bw)
    return out.reshape(b, s, d)
```
